```python
import os as _os
_os.environ.setdefault("JAX_PLATFORMS", "cpu")
import jax
import jax.numpy as jnp

def _softmax(x, axis=-1):
    return jax.nn.softmax(x, axis=axis)
def _gelu(x):
    return jax.nn.gelu(x, approximate=True)
def _silu(x):
    return jax.nn.silu(x)
def _sigmoid(x):
    return jax.nn.sigmoid(x)
def _layernorm(x, axis=-1, eps=1e-5):
    m = jnp.mean(x, axis=axis, keepdims=True)
    v = jnp.var(x, axis=axis, keepdims=True)
    return (x - m) / jnp.sqrt(v + eps)
def _scatter_add(tgt, idx, src, axis=0):
    return tgt.at[idx].add(src)
def _segment_sum(src, seg, n):
    return jax.ops.segment_sum(src, seg, n)
class _Rng:
    def __init__(self, key):
        self._k = key
    def _next(self):
        self._k, sub = jax.random.split(self._k)
        return sub
    def normal(self, shape):
        return jax.random.normal(self._next(), shape, dtype=jnp.bfloat16)
    def randint(self, lo, hi, shape):
        return jax.random.randint(self._next(), shape, lo, hi, dtype=jnp.int32)
    def uniform(self, shape, lo=0.0, hi=1.0):
        return jax.random.uniform(self._next(), shape, jnp.bfloat16, lo, hi)
    def permutation(self, n):
        return jax.random.permutation(self._next(), n)


kernel_name = 'parallel_sum__softmax_full_mha__swiglu_ffn__prompt'

def setup_inputs():
    _rng = _Rng(jax.random.key(int.from_bytes(__import__("os").urandom(4), "little")))
    _w = (lambda a: (lambda t: t.astype(jnp.bfloat16) if jnp.issubdtype(t.dtype, jnp.floating) else t)(jnp.asarray(a)))
    def _A_setup():
        B, S, D = 1, 2048, 640
        return {
            "x": _w((lambda *s: _rng.normal(s) * 0.05)(B, S, D)),
            "wqkv": _w((lambda *s: _rng.normal(s) * 0.1)(D, 3 * D)),
            "wo": _w((lambda *s: _rng.normal(s) * 0.05)(D, D)),
        }
    _A_in = _A_setup()

    def _B_setup():
        B, S, D, F = 1, 2048, 640, 1536
        return {
            "x": _w((lambda *s: _rng.normal(s) * 0.05)(B, S, D)),
            "w_gate": _w((lambda *s: _rng.normal(s) * 0.05)(D, F)),
            "w_up": _w((lambda *s: _rng.normal(s) * 0.05)(D, F)),
            "w_down": _w((lambda *s: _rng.normal(s) * 0.05)(F, D)),
        }
    _B_in = _B_setup()

    return {
        "A_x": _A_in["x"],
        "A_wqkv": _A_in["wqkv"],
        "A_wo": _A_in["wo"],
        "B_x": _B_in["x"],
        "B_w_gate": _B_in["w_gate"],
        "B_w_up": _B_in["w_up"],
        "B_w_down": _B_in["w_down"],
    }

def reference(A_x, A_wqkv, A_wo, B_x, B_w_gate, B_w_up, B_w_down):
    def _A_ref(x, wqkv, wo):
        B, S, D = x.shape
        H = 32; Dh = D // H
        qkv = (lambda x, *d: x.transpose(*d))((x @ wqkv).reshape(B, S, 3, H, Dh), 2, 0, 3, 1, 4)
        q, k, v = qkv[0], qkv[1], qkv[2]
        scale = Dh ** -0.5
        scores = jnp.einsum("bhqd,bhkd->bhqk", q, k) * scale
        p = _softmax(scores, axis=-1)
        o = jnp.einsum("bhqk,bhkd->bhqd", p, v)
        return (lambda x, *d: x.transpose(*d))(o, 0, 2, 1, 3).reshape(B, S, D) @ wo

    def _B_ref(x, w_gate, w_up, w_down):
        g = _silu(x @ w_gate)
        u = x @ w_up
        return (g * u) @ w_down

    x = A_x
    xn = _layernorm(x, axis=-1)
    return x + _A_ref(xn, A_wqkv, A_wo) + _B_ref(xn, B_w_gate, B_w_up, B_w_down)
```

```python
import jax
import jax.numpy as jnp
from jax import lax
from jax.experimental import pallas as pl
from jax.experimental.pallas import tpu as pltpu

S, D, F = 2048, 640, 1536
H, DH = 32, 20
LANES = 128
NMXU = 4
NKT = D // LANES
TQ = 512
NL = TQ // LANES
NQ = S // TQ
KC = 128
NC = S // KC
RC = 512
NR = S // RC
LS, LS0 = 16, 64
ES = 256
NES = TQ // ES
VP = 24
VPP = 32
VR = 16
EPS = 1e-5
QSCALE = (DH ** -0.5) * 1.4426950408889634
NN = (((1,), (0,)), ((), ()))
NT = (((1,), (1,)), ((), ()))
TN = (((0,), (0,)), ((), ()))
UNROLL = 2 * NQ
N_ITEMS = NQ * H
NB = N_ITEMS // UNROLL
FR = S // NB

NJ = 13
NJP = 16
GS = 3
SKEW = 1
MAX_DIST = 2
KB_DIST = 3
KB_END = 4
FFN_WEIGHT = 1.1

f32 = jnp.float32
bf16 = jnp.bfloat16
u32 = jnp.uint32

JSET = list(range(NC - NJ, NC))
VTASKS = [(j, min(GS, NJ - j), l) for j in range(0, NJ, GS) for l in range(NL)]
STRADDLE = [h for h in range(H) if (h * DH) // LANES != (h * DH + DH - 1) // LANES]


def _ffn_slots():
    nf = F // LANES
    tiles = []
    for a in range(nf):
        tiles += [('G', a, k) for k in range(NKT)] + [('U', a, k) for k in range(NKT)]
    tiles += [('D', n, k) for n in range(NKT) for k in range(nf)]
    groups = [tiles[i:i + NMXU] for i in range(0, len(tiles), NMXU)]
    slots, i = {}, 0
    for u in range(UNROLL):
        cnt = -(-(len(groups) - i) // (UNROLL - u))
        for c in [0, 1] + [1 + (j * (NC - 1)) // (cnt - 1) for j in range(1, cnt - 1)]:
            slots[u * NC + c] = groups[i]
            i += 1
    assert i == len(groups)
    return slots


FSLOTS = _ffn_slots()


def _vpu_slots(u):
    subs = [(ti, d) for ti in range(len(VTASKS)) for d in range(DH)]
    slots = list(range(SKEW if u == 0 else 0, NC))
    w = [1.0 + FFN_WEIGHT * ((u * NC + c - SKEW) in FSLOTS) for c in slots]
    cum = [sum(w[:k + 1]) / sum(w) for k in range(len(slots))]
    plan = {}
    tot, acc = sum(VTASKS[ti][1] for ti, _ in subs), 0.0
    for sub in subs:
        x = (acc + 0.5 * VTASKS[sub[0]][1]) / tot
        acc += VTASKS[sub[0]][1]
        plan.setdefault(slots[min(i for i in range(len(slots)) if cum[i] >= x)], []).append(sub)
    return plan


VSL = [_vpu_slots(u) for u in range(UNROLL)]


def _kb_slice(slot):
    nslot = NQ * (NC - SKEW) - KB_END
    if slot >= nslot:
        return []
    lo, hi = (slot * NJ * DH) // nslot, ((slot + 1) * NJ * DH) // nslot
    return [(d, max(lo - d * NJ, 0), min(hi - d * NJ, NJ)) for d in range(lo // NJ, (hi - 1) // NJ + 1)]


def _head_slot(h):
    if h in STRADDLE:
        return NKT, STRADDLE.index(h) * DH
    return (h * DH) // LANES, (h * DH) % LANES


def _pack(x):
    return pltpu.bitcast(x.astype(bf16), u32)


def _unpack(x):
    return pltpu.bitcast(x, bf16)


def _mul(i, n):
    return i * n if isinstance(i, int) else pl.multiple_of(i * n, n)


def _kernel(x_hbm, wqkv_hbm, wo_hbm, wg_hbm, wu_hbm, wd_hbm, o_hbm,
            x_ref, wqv_ref, wk_ref, wo_ref, wg_ref, wu_ref, wd_ref, out_ref,
            wg32_ref, wu32_ref, wd32_ref, wqvt_ref, xn_ref, k_ref, kv_ref, kba_ref, kbb_ref, qm_ref, qf_ref,
            vt_ref, ot_ref, sa_ref, sb_ref, res_ref,
            flag_ref, tile_ref, pos_ref, in_sems, x_sems, o_sems):
    flag_ref[0] = 0
    for h in range(H):
        tile_ref[h] = _head_slot(h)[0]
        pos_ref[h] = _head_slot(h)[1]

    def x_copy(r):
        r0 = _mul(r, RC)
        return pltpu.make_async_copy(x_hbm.at[pl.ds(r0, RC)], x_ref.at[pl.ds(r0, RC)], x_sems.at[r])

    wk_copy = pltpu.make_async_copy(wqkv_hbm.at[:, pl.ds(D, D)], wk_ref, in_sems.at[0])
    wq_copy = pltpu.make_async_copy(wqkv_hbm.at[:, pl.ds(0, D)], wqv_ref.at[:, pl.ds(0, D)], in_sems.at[1])
    wv_copy = pltpu.make_async_copy(wqkv_hbm.at[:, pl.ds(2 * D, D)], wqv_ref.at[:, pl.ds(D, D)], in_sems.at[2])
    late_copies = [pltpu.make_async_copy(src, dst, in_sems.at[3 + i]) for i, (src, dst) in enumerate(
        [(wg_hbm, wg_ref), (wu_hbm, wu_ref), (wd_hbm, wd_ref), (wo_hbm, wo_ref)])]
    x_copy(0).start()
    wk_copy.start()
    x_copy(1).start()
    wq_copy.start()
    wv_copy.start()
    for r in range(2, NR):
        x_copy(r).start()

    def layernorm(r, ls):
        for j in range(RC // ls):
            r0 = r * RC + j * ls if isinstance(r, int) else pl.multiple_of(r * RC + j * ls, ls)
            x = x_ref[pl.ds(r0, ls), :].astype(f32)
            mu = jnp.mean(x, axis=-1, keepdims=True)
            xc = x - mu
            var = jnp.mean(xc * xc, axis=-1, keepdims=True)
            xn_ref[pl.ds(r0, ls), :] = (xc * lax.rsqrt(var + EPS)).astype(bf16)

    def zero_fill(qb, c):
        for h in range(H):
            w0 = _head_slot(h)[1] // 16 * 16
            if w0 > 0:
                qm_ref[qb, h, 0:w0 // 2, :] = jnp.zeros((w0 // 2, TQ), u32)
            if w0 + 32 < LANES:
                qm_ref[qb, h, w0 // 2 + 16:LANES // 2, :] = jnp.zeros((LANES // 2 - w0 // 2 - 16, TQ), u32)
        sb_ref[pl.ds(_mul(qb, S // NQ), S // NQ), :] = jnp.zeros((S // NQ, TQ), f32)
        return c

    lax.fori_loop(0, NQ, zero_fill, 0)

    x_copy(0).wait()
    layernorm(0, LS0)
    wk_copy.wait()

    lane_k = lax.broadcasted_iota(jnp.int32, (RC, LANES), 1)

    def kproj(r, with_xpose):
        @pl.when(r + 1 < NR)
        def _():
            x_copy(r + 1).wait()

        if with_xpose:
            c0 = pl.multiple_of((r - NR // 2) * D, D)
            wqvt_ref[pl.ds(c0, D), :] = wqv_ref[:, pl.ds(c0, D)].astype(f32).T.astype(bf16)

        k = jnp.dot(xn_ref[pl.ds(_mul(r, RC), RC), :], wk_ref[...], preferred_element_type=f32)
        tiles = [k[:, g * LANES:(g + 1) * LANES] for g in range(NKT)]
        extra = jnp.zeros((RC, LANES), f32)
        for s, h in enumerate(STRADDLE):
            g = (h * DH) // LANES
            off = (h * DH) % LANES
            joined = jnp.where(lane_k >= off, tiles[g], tiles[g + 1])
            moved = pltpu.roll(joined, (s * DH - off) % LANES, 1)
            extra = jnp.where((lane_k >= s * DH) & (lane_k < (s + 1) * DH), moved, extra)
        for g, tile in enumerate(tiles + [extra]):
            k_ref[g, pl.ds(_mul(r, RC // 2), RC // 2), :] = _pack(tile)
        layernorm(jnp.minimum(r + 1, NR - 1), LS)

    def kproj_a(r, c):
        kproj(r, False)
        return c

    def kproj_b(r, c):
        kproj(r, True)
        return c

    lax.fori_loop(0, NR // 2, kproj_a, 0)
    wq_copy.wait()
    wv_copy.wait()
    for c in late_copies:
        c.start()
    lax.fori_loop(NR // 2, NR, kproj_b, 0)

    for ji in range(NJ):
        r0 = JSET[ji] * KC // 2
        kv_ref[:, ji * (VR // 2):(ji + 1) * (VR // 2), :] = k_ref[:, r0:r0 + VR // 2, :]

    def build_kb(h, runs, kb_ref, never=None, gate=None):
        g = tile_ref[h]
        pos = pos_ref[h]
        done = None
        for d, j0, j1 in runs:
            k = kv_ref[g, j0 * (VR // 2):j1 * (VR // 2), :]
            if gate is not None:
                k = jnp.where(never, jnp.concatenate([pltpu.bitcast(gate, u32)] * (j1 - j0), axis=0), k)
            kb = jnp.take_along_axis(k, jnp.full(k.shape, pos + d, jnp.int32), axis=1, mode='promise_in_bounds')
            kb = _unpack(kb).astype(f32)
            kb_ref[d, j0 * VR:j1 * VR, :] = kb
            if gate is not None:
                for r in range(kb.shape[0] // 8):
                    done = kb[8 * r:8 * r + 8] if done is None else jnp.maximum(done, kb[8 * r:8 * r + 8])
        return done

    row_w = lax.broadcasted_iota(jnp.int32, (32, TQ), 0)
    row8 = lax.broadcasted_iota(jnp.int32, (8, TQ), 0)

    def qvproj(r, repack):
        if repack:
            hf = r - NQ // 2
            for src, dst, n in ((wg_ref, wg32_ref, D // 2), (wu_ref, wu32_ref, D // 2), (wd_ref, wd32_ref, F // 2)):
                dst[pl.ds(_mul(hf, n // 2), n // 2), :] = pltpu.bitcast(src[pl.ds(_mul(hf, n), n), :], u32)
        build_kb(0, [(r * (DH // NQ) + dd, 0, NJ) for dd in range(DH // NQ)], kba_ref)
        qvt = lax.dot_general(wqvt_ref[...], xn_ref[pl.ds(_mul(r, TQ), TQ), :], NT, preferred_element_type=f32)
        for h in range(H):
            pos = _head_slot(h)[1]
            w0 = pos // 16 * 16
            lo = pos - w0
            src = h * DH - lo
            win = qvt[src:src + 32] * QSCALE
            win = jnp.where((row_w >= lo) & (row_w < lo + DH), win, 0.0)
            qm_ref[r, h, w0 // 2:w0 // 2 + 16, :] = _pack(win)
            qf_ref[r, h] = (qvt[h * DH:h * DH + 24] * QSCALE).astype(bf16).astype(f32)
        for h in range(H):
            lo = D + h * DH
            hi = min(lo + 16, 2 * D - 8)
            tail = qvt[hi:hi + 8]
            if hi != lo + 16:
                tail = pltpu.roll(tail, 8 - (lo + 16 - hi), 0)
            tail = jnp.where(row8 < DH - 16, tail, jnp.where(row8 == DH - 16, 1.0, 0.0))
            vt = jnp.concatenate([qvt[lo:lo + 16], tail], axis=0)
            for j in range(TQ // KC):
                vt_ref[r * (TQ // KC) + j, h * VPP:h * VPP + VP, :] = vt[:, j * KC:(j + 1) * KC]

    def qvproj_a(r, c):
        qvproj(r, False)
        return c

    def qvproj_b(r, c):
        qvproj(r, True)
        return c

    lax.fori_loop(0, NQ // 2, qvproj_a, 0)
    for c in late_copies:
        c.wait()
    lax.fori_loop(NQ // 2, NQ, qvproj_b, 0)

    def load_q(t):
        qb, h = t % NQ, t // NQ
        return tile_ref[h], qm_ref.at[qb, h], qf_ref.at[qb, h]

    def qk_chunk(q, c, s_ref, m8):
        nv = VR * JSET.count(c)
        s = jnp.dot(_unpack(k_ref[q[0], pl.ds((c * KC + nv) // 2, (KC - nv) // 2), :]), _unpack(q[1][...]),
                    preferred_element_type=f32)
        s_ref[pl.ds(c * KC + nv, KC - nv), :] = s
        cm = jnp.max(s.reshape((KC - nv) // 8, 8, TQ), axis=0)
        return s, (cm if m8 is None else jnp.maximum(m8, cm))

    def pv_chunk(h, c, s_ref, m, acc):
        s = s_ref[pl.ds(c * KC, KC), :].reshape(KC // 8, 8, TQ)
        p = jnp.exp2(s - m[None]).reshape(KC, TQ).astype(bf16)
        d = lax.dot_general(vt_ref[c, pl.ds(_mul(h, VPP), VP), :], p, NN, precision=lax.Precision.DEFAULT,
                            preferred_element_type=f32)
        return d if acc is None else acc + d

    def store_o(t, parity, acc):
        ot_ref[t % NQ, t // (2 * NQ), parity * DH:(parity + 1) * DH, :] = acc[:DH] * (1.0 / acc[DH:DH + 1])

    kbs = (kba_ref, kbb_ref)
    bufs = (sa_ref, sb_ref)
    last_item = N_ITEMS - 1

    m8 = None
    for c in range(SKEW):
        _, m8 = qk_chunk(load_q(0), c, sa_ref, m8)

    def block(i, carry):
        m_cur, m8 = carry
        never = flag_ref[0] != 0
        f0 = pl.multiple_of(i * FR, FR)
        xn_f = xn_ref[pl.ds(f0, FR), :]
        xn_tiles = [xn_f[:, k * LANES:(k + 1) * LANES] for k in range(NKT)]
        hids, part, kb_done, hist = [], {}, [], []

        def do_ffn(n):
            ticks = []
            for kind, a, k in FSLOTS.get(n, []):
                lhs = hids[k] if kind == 'D' else xn_tiles[k]
                w_ref = {'G': wg32_ref, 'U': wu32_ref, 'D': wd32_ref}[kind]
                y = jnp.dot(lhs, _unpack(w_ref[k * 64:(k + 1) * 64, a * LANES:(a + 1) * LANES]),
                            preferred_element_type=f32)
                if not ticks:
                    ticks = [(y, r) for r in range(FR // 8)]
                if k > 0:
                    y = part[kind] + y
                elif kind == 'D':
                    y = x_ref[pl.ds(f0, FR), a * LANES:(a + 1) * LANES].astype(f32) + y
                part[kind] = y
                if kind == 'U' and k == NKT - 1:
                    g = part['G']
                    hids.append((g * (0.5 * jnp.tanh(0.5 * g) + 0.5) * y).astype(bf16))
                if kind == 'D' and k == F // LANES - 1:
                    res_ref[pl.ds(f0, FR), a * LANES:(a + 1) * LANES] = y
            return ticks

        mv = [None] * NL
        q = load_q(UNROLL * i)
        for u in range(UNROLL):
            t = UNROLL * i + u
            tp = jnp.where(t > 0, t - 1, NQ) if u == 0 else t - 1
            h_prev = tp // NQ
            h_new = jnp.minimum(t // NQ + 1, H - 1)
            acc = None
            for c in range(NC):
                n = u * NC + c
                ticks = do_ffn(n)
                m_use = jnp.where(never, hist[n - MAX_DIST], m_cur) if n >= MAX_DIST else m_cur
                if n >= KB_DIST and kb_done[n - KB_DIST] is not None:
                    m_use = jnp.concatenate(
                        [jnp.where(never, kb_done[n - KB_DIST], m_use[:, :LANES]), m_use[:, LANES:]], axis=1)
                e, cq = divmod(n + SKEW, NC)
                if cq == 0:
                    m_all = jnp.maximum(m8, jnp.concatenate(mv, axis=1))
                    m_next = jnp.broadcast_to(jnp.max(m_all, axis=0, keepdims=True), (8, TQ))
                    m8 = None
                    mv = [None] * NL
                    q = load_q(jnp.minimum(t + 1, last_item))
                s, m8 = qk_chunk(q, cq, bufs[e % 2], m8)
                ticks += [(s, r) for r in range(s.shape[0] // 8)]

                subs = VSL[e].get(cq, []) if e < UNROLL else []
                for k, (ti, d) in enumerate(subs):
                    j0, gs, l = VTASKS[ti]
                    if k == 0 or d == 0:
                        d_lo, d_hi = d, max(dd for tt, dd in subs if tt == ti) + 1
                        kall = kbs[(e // NQ) % 2][d_lo:d_hi, j0 * VR:(j0 + gs) * VR, :]
                    src, r = ticks[(k * len(ticks)) // len(subs)]
                    row = jnp.broadcast_to(q[2][d:d + 1, l * LANES:(l + 1) * LANES], (8, LANES))
                    row = jnp.where(never, src[8 * r:8 * r + 8, :LANES], row)
                    prod = kall[d - d_lo].reshape(gs * VR // 8, 8, LANES) * row[None]
                    vacc = prod if d == 0 else vacc + prod
                    if d == DH - 1:
                        cm = jnp.max(vacc, axis=0)
                        sv = vacc.reshape(gs * VR, LANES)
                        for a in range(gs):
                            r0 = JSET[j0 + a] * KC
                            bufs[e % 2][r0:r0 + VR, l * LANES:(l + 1) * LANES] = sv[VR * a:VR * (a + 1)]
                        mv[l] = cm if mv[l] is None else jnp.maximum(mv[l], cm)

                runs = _kb_slice((u % NQ) * (NC - SKEW) + c) if e == u else []
                done = None
                if runs:
                    done = build_kb(h_new, runs, kbs[(u // NQ + 1) % 2], never,
                                    hist[n - 1][:, :LANES] if n >= 1 else None)
                kb_done.append(done if u < NQ else None)
                hist.append(m8)
                acc = pv_chunk(h_prev, c, bufs[(u + 1) % 2], m_use, acc)
            m_cur = m_next
            store_o(tp, ((u - 1) // NQ) % 2, acc)
        return m_cur, m8

    m_last, _ = lax.fori_loop(0, NB, block, (jnp.zeros((8, TQ), f32), m8))

    def out_rows(qb, j):
        r0 = qb * TQ + j * ES
        return pl.ds(r0 if isinstance(qb, int) else pl.multiple_of(r0, ES), ES)

    def o_copy(qb, j):
        return pltpu.make_async_copy(out_ref.at[out_rows(qb, j)], o_hbm.at[out_rows(qb, j)], o_sems.at[qb * NES + j])

    def epi_piece(qb, j):
        ot = ot_ref[qb, :, :, j * ES:(j + 1) * ES].reshape(D, ES).astype(bf16)
        attn = lax.dot_general(ot, wo_ref[...], TN, preferred_element_type=f32)
        out_ref[out_rows(qb, j), :] = (res_ref[out_rows(qb, j), :] + attn).astype(out_ref.dtype)

    acc = None
    for c in range(NC):
        if c % (NC // NES) == 0:
            epi_piece(0, c // (NC // NES))
        acc = pv_chunk(H - 1, c, bufs[last_item % 2], m_last, acc)
    store_o(last_item, (H - 1) % 2, acc)
    for j in range(NES):
        o_copy(0, j).start()

    def epi(qb, c):
        for j in range(NES):
            epi_piece(qb, j)
            o_copy(qb, j).start()
        return c

    lax.fori_loop(1, NQ, epi, 0)
    for qb in range(NQ):
        for j in range(NES):
            o_copy(qb, j).wait()


@jax.jit
def pallas_parallel_sum__softmax_full_mha__swiglu_ffn__prompt_kernel(
        A_x, A_wqkv, A_wo, B_x, B_w_gate, B_w_up, B_w_down):
    del B_x
    args = (A_x.reshape(S, D), A_wqkv, A_wo, B_w_gate, B_w_up, B_w_down)
    out = pl.pallas_call(
        _kernel,
        in_specs=[pl.BlockSpec(memory_space=pl.ANY)] * len(args),
        out_specs=pl.BlockSpec(memory_space=pl.ANY),
        out_shape=jax.ShapeDtypeStruct((S, D), bf16),
        scratch_shapes=[
            pltpu.VMEM((S, D), bf16),
            pltpu.VMEM((D, 2 * D), bf16),
            pltpu.VMEM((D, D), bf16),
            pltpu.VMEM((D, D), bf16),
            pltpu.VMEM((D, F), bf16),
            pltpu.VMEM((D, F), bf16),
            pltpu.VMEM((F, D), bf16),
            pltpu.VMEM((S, D), bf16),
            pltpu.VMEM((D // 2, F), u32),
            pltpu.VMEM((D // 2, F), u32),
            pltpu.VMEM((F // 2, D), u32),
            pltpu.VMEM((2 * D, D), bf16),
            pltpu.VMEM((S, D), bf16),
            pltpu.VMEM((NKT + 1, S // 2, LANES), u32),
            pltpu.VMEM((NKT + 1, NJP * VR // 2, LANES), u32),
            pltpu.VMEM((DH, NJP * VR, LANES), f32),
            pltpu.VMEM((DH, NJP * VR, LANES), f32),
            pltpu.VMEM((NQ, H, LANES // 2, TQ), u32),
            pltpu.VMEM((NQ, H, 24, TQ), f32),
            pltpu.VMEM((NC, H * VPP, KC), f32),
            pltpu.VMEM((NQ, H // 2, 2 * DH, TQ), f32),
            pltpu.VMEM((S, TQ), f32),
            pltpu.VMEM((S, TQ), f32),
            pltpu.VMEM((S, D), f32),
            pltpu.SMEM((1,), jnp.int32),
            pltpu.SMEM((H,), jnp.int32),
            pltpu.SMEM((H,), jnp.int32),
            pltpu.SemaphoreType.DMA((7,)),
            pltpu.SemaphoreType.DMA((NR,)),
            pltpu.SemaphoreType.DMA((NQ * NES,)),
        ],
        compiler_params=pltpu.CompilerParams(vmem_limit_bytes=110 * 2 ** 20),
        name="fused",
    )(*args)
    return out.reshape(1, S, D)
```
